```python
import os as _os
_os.environ.setdefault("JAX_PLATFORMS", "cpu")
import jax
import jax.numpy as jnp

def _softmax(x, axis=-1):
    return jax.nn.softmax(x, axis=axis)
def _gelu(x):
    return jax.nn.gelu(x, approximate=True)
def _silu(x):
    return jax.nn.silu(x)
def _sigmoid(x):
    return jax.nn.sigmoid(x)
def _layernorm(x, axis=-1, eps=1e-5):
    m = jnp.mean(x, axis=axis, keepdims=True)
    v = jnp.var(x, axis=axis, keepdims=True)
    return (x - m) / jnp.sqrt(v + eps)
def _scatter_add(tgt, idx, src, axis=0):
    return tgt.at[idx].add(src)
def _segment_sum(src, seg, n):
    return jax.ops.segment_sum(src, seg, n)
class _Rng:
    def __init__(self, key):
        self._k = key
    def _next(self):
        self._k, sub = jax.random.split(self._k)
        return sub
    def normal(self, shape):
        return jax.random.normal(self._next(), shape, dtype=jnp.bfloat16)
    def randint(self, lo, hi, shape):
        return jax.random.randint(self._next(), shape, lo, hi, dtype=jnp.int32)
    def uniform(self, shape, lo=0.0, hi=1.0):
        return jax.random.uniform(self._next(), shape, jnp.bfloat16, lo, hi)
    def permutation(self, n):
        return jax.random.permutation(self._next(), n)


kernel_name = 'parallel_sum__ssm_conv_h3__dense_activation_silu__prompt'

def setup_inputs():
    _rng = _Rng(jax.random.key(int.from_bytes(__import__("os").urandom(4), "little")))
    _w = (lambda a: (lambda t: t.astype(jnp.bfloat16) if jnp.issubdtype(t.dtype, jnp.floating) else t)(jnp.asarray(a)))
    def _A_setup():
        B, S, D = 1, 2048, 448
        ks = 4
        return {
            "q": _w((lambda *s: _rng.normal(s) * 0.05)(B, S, D)),
            "k": _w((lambda *s: _rng.normal(s) * 0.2)(B, S, D)),
            "v": _w((lambda *s: _rng.normal(s) * 0.2)(B, S, D)),
            "shift_k": _w((lambda *s: _rng.normal(s) * 0.2)(D, ks) * 0.5),
            "ssm_k": _w((lambda *s: _rng.normal(s) * 0.2)(D, S) * (1.0 / S ** 0.5)),
            "ssm_D": _w((lambda *s: _rng.normal(s) * 0.2)(D)),
        }
    _A_in = _A_setup()

    def _B_setup():
        B, S, D, F = 1, 2048, 448, 1792
        return {
            "x": _w((lambda *s: _rng.normal(s) * 0.05)(B, S, D)),
            "w1": _w((lambda *s: _rng.normal(s) * 0.05)(D, F) * (D ** -0.5)),
            "w2": _w((lambda *s: _rng.normal(s) * 0.05)(F, D) * (F ** -0.5)),
        }
    _B_in = _B_setup()

    return {
        "A_q": _A_in["q"],
        "A_k": _A_in["k"],
        "A_v": _A_in["v"],
        "A_shift_k": _A_in["shift_k"],
        "A_ssm_k": _A_in["ssm_k"],
        "A_ssm_D": _A_in["ssm_D"],
        "B_x": _B_in["x"],
        "B_w1": _B_in["w1"],
        "B_w2": _B_in["w2"],
    }

def reference(A_q, A_k, A_v, A_shift_k, A_ssm_k, A_ssm_D, B_x, B_w1, B_w2):
    def _A_ref(q, k, v, shift_k, ssm_k, ssm_D):
        B, S, D = q.shape
        ks = shift_k.shape[-1]
        k_pad = jnp.pad(k, ((0, 0), (ks - 1, 0), (0, 0)))
        k_shift = jnp.zeros_like(k)
        for t in range(ks):
            k_shift = k_shift + k_pad[:, t:t + S, :] * shift_k[:, ks - 1 - t][None, None, :]
        kv = k_shift * v
        L = 2 * S
        kv_pad = jnp.pad(kv, ((0, 0), (0, S), (0, 0)))
        kf_pad = jnp.pad(ssm_k, ((0, 0), (0, S)))
        kv_f = (lambda x, axes=(-2,-1): jnp.fft.rfft2(x.astype(jnp.float32), axes=axes))(kv_pad[:, None, :, :], axes=(1, 2))
        kf_f = (lambda x, axes=(-2,-1): jnp.fft.rfft2(x.astype(jnp.float32), axes=axes))(kf_pad[:, None, :], axes=(1, 2))
        kf_f = (lambda x, *d: x.transpose(*d))(kf_f, 1, 2, 0)
        y_f = kv_f * kf_f[None, :, :, :]
        y = (lambda x, s, axes=(-2,-1): jnp.fft.irfft2(x, s=s, axes=axes).astype(jnp.bfloat16))(y_f, (1, L), axes=(1, 2))[:, 0, :S, :]
        y = y + kv * ssm_D[None, None, :]
        return q * y

    def _B_ref(x, w1, w2):
        h = jnp.einsum("bsd,df->bsf", x, w1)
        h = _silu(h)
        out = jnp.einsum("bsf,fd->bsd", h, w2)
        return out

    x = A_q
    xn = _layernorm(x, axis=-1)
    return x + _A_ref(xn, A_k, A_v, A_shift_k, A_ssm_k, A_ssm_D) + _B_ref(xn, B_w1, B_w2)
```

```python
import os
import jax
import jax.numpy as jnp
import numpy as np
import jax.experimental.pallas as pl
import jax.experimental.pallas.tpu as pltpu

D, S, F = 448, 2048, 1792
B = 128
NB = S // B
NS = NB // 2
NF = F // B
f32 = jnp.float32
bf16 = jnp.bfloat16
u32 = jnp.uint32

def _consts():
    n = np.arange(B)[:, None].astype(np.float64)
    f = np.arange(B)[None, :].astype(np.float64)
    w = 2 * np.pi * (f + 0.5) / (2 * B)
    sig = np.where(np.arange(B) % 2 == 0, 1.0, -1.0)[None, :]
    Fm = np.stack([np.cos(w * n), -np.sin(w * n) * sig])
    Gm = np.concatenate([(np.cos(w * n)).T, (-np.sin(w * n) * sig).T], axis=0) / B
    return Fm.astype(np.float32), Gm.astype(np.float32)
_FM, _GM = _consts()

def ldb(ref, idx, r):
    return pltpu.bitcast(ld32(ref, idx, r), bf16)
def ld32(ref, idx, r):
    v = ref.bitcast(u32)
    rr = slice(r.start // 2, r.stop // 2)
    return v[(*idx, rr, slice(None))]

NU = 28
L2 = int(os.environ.get('L2', 6))
NOREG = os.environ.get('NOREG', '')
SCOPES = int(os.environ.get('SCOPES', 0))
CH = D // NU
FR = F // NU
DR = D // 4

def kern(qT_h, kT_h, vT_h, skT_h, ssmk_h, sD_h, w1_h, w2T_h, Fm_h, Gm_h, oT_h,
         qb, kb, vb, sb, w1b, w2o, skT, sD, Fm, Gm, sems,
         w1T, skb, db, Ua, Ub, Us, Ka, Kb, Kc, hT, Kpr, Kpi, xnb, yb, acc):
    def cp_blk(src, dst, i, j, sem):
        return pltpu.make_async_copy(src.at[:, pl.ds(B * i, B)], dst.at[j], sems.at[sem])
    def cp_in(n, i):
        src, dst = ((qT_h, qb), (kT_h, kb), (vT_h, vb), (ssmk_h, sb))[n]
        return cp_blk(src, dst, i, i, i * 4 + n)
    def cp_w(n, c):
        src, dst = ((w1_h, w1b), (w2T_h, w2o))[n]
        return cp_blk(src, dst, c, c, 64 + n * NF + c)
    def cp_out(i):
        return pltpu.make_async_copy(w2o.at[NF + i], oT_h.at[:, pl.ds(B * i, B)], sems.at[64 + 2 * NF + i])

    scope = [None]
    def enter(name):
        if not SCOPES:
            return
        if scope[0] is not None:
            scope[0].__exit__(None, None, None)
        scope[0] = jax.named_scope(name) if name else None
        if name:
            scope[0].__enter__()
    enter('p_start')
    small = [pltpu.make_async_copy(src, dst, sems.at[108 + n]) for n, (src, dst) in
             enumerate(((skT_h, skT), (sD_h, sD), (Fm_h, Fm), (Gm_h, Gm)))]
    order = [cp_in(0, 0), cp_in(0, 1), cp_w(0, 0), cp_w(0, 1)] + small + [cp_w(0, 2), cp_w(0, 3), cp_w(1, 0), cp_w(1, 1)]
    order += [cp_in(n, i) for n in (1, 2, 3) for i in range(2)]
    for kc in range(2, 7):
        order += [cp_w(0, 2 * kc), cp_w(0, 2 * kc + 1), cp_w(1, 2 * kc - 2), cp_w(1, 2 * kc - 1)]
    order += [cp_w(1, 12), cp_w(1, 13), cp_in(0, 2), cp_in(0, 3)] + [cp_in(n, i) for n in (1, 2, 3) for i in (2, 3)]
    for i in range(4, NB, 2):
        order += [cp_in(n, i + b) for n in range(4) for b in range(2)]
    for c in order:
        c.start()

    def smallprep():
        sk = skT[...].astype(f32)
        for j in range(4):
            skb[j] = jnp.broadcast_to(sk[j:j + 1, :], (B, D)).T
        db[...] = jnp.broadcast_to(sD[...].astype(f32)[None, :], (B, D)).T
    lane = jax.lax.broadcasted_iota(jnp.int32, (CH // 2, B), 1)

    def ln(i):
        x = qb[i].astype(f32)
        mu = jnp.sum(x, axis=0, keepdims=True) * (1.0 / D)
        xc = x - mu
        var = jnp.sum(xc * xc, axis=0, keepdims=True) * (1.0 / D)
        xn = xc * jax.lax.rsqrt(var + 1e-5)
        xnb[i % 4, :D, :] = xn.astype(bf16)

    def fmat():
        return jnp.concatenate([ldb(Fm, (0,), slice(0, B)), ldb(Fm, (1,), slice(0, B))], axis=1)

    def dft_kv(s, u):
        r = slice(CH * u, CH * (u + 1))
        kvs = []
        for b in range(2):
            i = 2 * s + b
            a0 = ld32(kb, (i,), r)
            ap = ld32(kb, (i - 1,), r) if i > 0 else jnp.zeros_like(a0)
            ks = pltpu.bitcast(a0, bf16).astype(f32) * skb[0, r, :]
            for j in range(1, 4):
                m = pltpu.roll(jnp.where(lane >= B - j, ap, a0), j, 1)
                ks = ks + pltpu.bitcast(m, bf16).astype(f32) * skb[j, r, :]
            kvs.append(ks * vb[i, r, :].astype(f32))
        T = jnp.dot(jnp.concatenate(kvs, axis=0).astype(bf16), fmat(), preferred_element_type=f32)
        for b in range(2):
            i = 2 * s + b
            ur, ui = T[b * CH:(b + 1) * CH, :B], T[b * CH:(b + 1) * CH, B:]
            Ua[i, r, :] = ur
            Ub[i, r, :] = ui
            Us[i, r, :] = ur + ui

    def dft_k(s, u):
        r = slice(CH * u, CH * (u + 1))
        lhs = pltpu.bitcast(jnp.concatenate([ld32(sb, (2 * s,), r), ld32(sb, (2 * s + 1,), r)], axis=0), bf16)
        T = jnp.dot(lhs, fmat(), preferred_element_type=f32)
        for b in range(2):
            i = 2 * s + b
            kr, ki = T[b * CH:(b + 1) * CH, :B], T[b * CH:(b + 1) * CH, B:]
            if i == 0:
                kr = kr + db[r, :]
                c, d = kr, ki
            elif b == 0:
                c = kr - Kpi[r, :]
                d = ki + Kpr[r, :]
            else:
                c = kr - pki
                d = ki + pkr
            pkr, pki = kr, ki
            Ka[i, r, :] = c
            Kb[i, r, :] = d - c
            Kc[i, r, :] = c + d
        Kpr[r, :] = pkr
        Kpi[r, :] = pki

    def mac(s, g):
        r = slice(8 * g, 8 * (g + 1))
        a = [None, None]
        k1 = (Ka[2 * s + 1, r, :], Kb[2 * s + 1, r, :], Kc[2 * s + 1, r, :])
        for j in range(2 * s + 2):
            ua, ub, us = Ua[j, r, :], Ub[j, r, :], Us[j, r, :]
            t = (k1[0] * us, k1[1] * ua, k1[2] * ub)
            a[1] = t if a[1] is None else tuple(x + y for x, y in zip(a[1], t))
            m0 = 2 * s - j
            if m0 >= 0:
                k1 = (Ka[m0, r, :], Kb[m0, r, :], Kc[m0, r, :])
                t = (k1[0] * us, k1[1] * ua, k1[2] * ub)
                a[0] = t if a[0] is None else tuple(x + y for x, y in zip(a[0], t))
        yr = jnp.concatenate([(a[b][0] - a[b][2]) for b in range(2)], axis=0)
        yi = jnp.concatenate([(a[b][0] + a[b][1]) for b in range(2)], axis=0)
        lhs = jnp.concatenate([yr, yi], axis=1).astype(bf16)
        y = jnp.dot(lhs, ldb(Gm, (), slice(0, 2 * B)), preferred_element_type=f32)
        for b in range(2):
            yb[(2 * s + b) % 4, r, :] = y[b * 8:(b + 1) * 8, :]

    def ffn1(s, u):
        r = slice(FR * u, FR * (u + 1))
        lhs = pltpu.bitcast(jnp.concatenate([ld32(w1T, (k,), r) for k in range(4)], axis=1), bf16)
        rhs = pltpu.bitcast(jnp.concatenate([ld32(xnb, ((2 * s + b) % 4,), slice(0, 4 * B)) for b in range(2)], axis=1), bf16)
        hh = jnp.dot(lhs, rhs, preferred_element_type=f32)
        for b in range(2):
            hb = hh[:, b * B:(b + 1) * B]
            hT[s % 2, b, r, :] = (hb + hb * jnp.tanh(hb)).astype(bf16)

    def ffn2(s, u):
        kc, q = u // 4, u % 4
        r = slice(DR * q, DR * (q + 1))
        fr = slice(2 * B * kc, 2 * B * (kc + 1))
        lhs = pltpu.bitcast(jnp.concatenate([ld32(w2o, (2 * kc + k,), r) for k in range(2)], axis=1), bf16)
        rhs = pltpu.bitcast(jnp.concatenate([ld32(hT, (s % 2, b), fr) for b in range(2)], axis=1), bf16)
        p = jnp.dot(lhs, rhs, preferred_element_type=f32)
        if kc == 0:
            acc[r, :] = p
        elif kc < 6:
            acc[r, :] = acc[r, :] + p
        else:
            for b in range(2):
                i = 2 * s + b
                tot = acc[r, b * B:(b + 1) * B] + p[:, b * B:(b + 1) * B]
                x = qb[i, r, :].astype(f32)
                xn = xnb[i % 4, r, :].astype(f32)
                w2o[NF + i, r, :] = (x + xn * yb[i % 4, r, :] + tot).astype(bf16)

    def w1prep(c):
        for k in range(4):
            blk = w1b[c, B * k:min(B * (k + 1), D), :].astype(f32) * 0.5
            if k == 3:
                blk = jnp.concatenate([blk, jnp.zeros((4 * B - D, B), f32)], axis=0)
            w1T[k, B * c:B * (c + 1), :] = blk.T.astype(bf16)

    T = NU * NS + L2
    ev = {t: dict(bar=[], pre=[], a=[], b=[]) for t in range(T)}
    def at(t, slot, fn, *args):
        ev[t][slot].append((fn, args))
    ev[0]['bar'] = [cp_w(0, 0), cp_w(0, 1)]
    at(0, 'pre', w1prep, 0); at(0, 'pre', w1prep, 1)
    ev[4]['bar'] = small + [cp_w(0, 2), cp_w(0, 3), cp_w(1, 0), cp_w(1, 1)]
    at(4, 'pre', w1prep, 2); at(4, 'pre', w1prep, 3); at(4, 'pre', smallprep)
    ev[8]['bar'] = [cp_in(n, i) for n in (1, 2, 3) for i in range(2)] + [cp_w(0, 4), cp_w(0, 5), cp_w(1, 2), cp_w(1, 3)]
    for k, t in enumerate((12, 16, 20, 24)):
        kc = 3 + k
        ev[t]['bar'] = [cp_w(0, 2 * kc), cp_w(0, 2 * kc + 1), cp_w(1, 2 * kc - 2), cp_w(1, 2 * kc - 1)]
    ev[24]['bar'] += [cp_w(1, 12), cp_w(1, 13), cp_in(0, 2), cp_in(0, 3)]
    for kc in range(2, 7):
        at(4 * kc, 'pre', w1prep, 2 * kc); at(4 * kc, 'pre', w1prep, 2 * kc + 1)
    ev[NU]['bar'] = [cp_in(n, i) for n in (1, 2, 3) for i in (2, 3)]
    for s in range(1, NS):
        bar = [cp_in(n, 2 * s + 2 + b) for n in range(4) for b in range(2)] if s + 1 < NS else []
        if s >= 2:
            bar += [cp_out(2 * s - 4), cp_out(2 * s - 3)]
        ev[NU * s + L2]['bar'] = bar
    for c in range(NU):
        td = {0: 8 + c // 2, 1: NU + c}
        tm = {0: 9 + c // 2, 1: NU + c + 1}
        for s in range(2, NS):
            td[s] = NU * (s - 1) + L2 + c
            tm[s] = NU * s + c
        for s in range(NS):
            at(td[s], 'a', dft_kv, s, c)
            at(td[s], 'b', dft_k, s, c)
    for c in range(NU):
        tm = {0: 9 + c // 2, 1: NU + c + 1}
        for s in range(2, NS):
            tm[s] = NU * s + c
        for s in range(NS):
            ev[tm[s]]['a'].insert(0, (mac, (s, 2 * c))) if False else ev[tm[s]].setdefault('m0', []).append((mac, (s, 2 * c)))
            ev[tm[s]].setdefault('m1', []).append((mac, (s, 2 * c + 1)))

    for i in range(4):
        xnb[i, D:, :] = jnp.zeros((4 * B - D, B), bf16)
    enter('p_qwait')
    for i in range(2):
        cp_in(0, i).wait()
    enter('p_ln')
    ln(0)
    ln(1)
    for t in range(T):
        s, u = t // NU, t % NU
        if u == 0:
            enter(f'step{s}')
        e = ev[t]
        for c in e['bar']:
            c.wait()
        for fn, args in e['pre']:
            fn(*args)
        if s < NS:
            ffn1(s, u)
        for fn, args in e.get('m0', []):
            fn(*args)
        for fn, args in e['a']:
            fn(*args)
        if t >= L2:
            s2, u2 = (t - L2) // NU, (t - L2) % NU
            ffn2(s2, u2)
            if u2 == NU - 1:
                cp_out(2 * s2).start()
                cp_out(2 * s2 + 1).start()
        for fn, args in e['b']:
            fn(*args)
        for fn, args in e.get('m1', []):
            fn(*args)
        if u == NU - 1 and s + 1 < NS:
            ln(2 * s + 2)
            ln(2 * s + 3)
    enter('epi')
    for i in range(NB - 4, NB):
        cp_out(i).wait()
    enter(None)

def pallas_parallel_sum__ssm_conv_h3__dense_activation_silu__prompt_kernel(A_q, A_k, A_v, A_shift_k, A_ssm_k, A_ssm_D, B_x, B_w1, B_w2):
    qT = A_q[0].T
    kT = A_k[0].T
    vT = A_v[0].T
    Fm = jnp.asarray(_FM, dtype=bf16)
    Gm = jnp.asarray(_GM, dtype=bf16)
    vm = pl.BlockSpec(memory_space=pltpu.VMEM)
    hb = pl.BlockSpec(memory_space=pltpu.HBM)
    blk = lambda n: pltpu.VMEM((n, D, B), bf16)
    outT = pl.pallas_call(
        kern,
        in_specs=[hb] * 10,
        out_specs=hb,
        out_shape=jax.ShapeDtypeStruct((D, S), A_q.dtype),
        scratch_shapes=[
            blk(NB), blk(NB), blk(NB), blk(NB), blk(NF), blk(NF + NB),
            pltpu.VMEM((4, D), bf16), pltpu.VMEM((D,), bf16), pltpu.VMEM((2, B, B), bf16), pltpu.VMEM((2 * B, B), bf16),
            pltpu.SemaphoreType.DMA((112,)),
            pltpu.VMEM((4, F, B), bf16),
            pltpu.VMEM((4, D, B), f32),
            pltpu.VMEM((D, B), f32),
        ] + [pltpu.VMEM((NB, D, B), f32)] * 6 + [
            pltpu.VMEM((2, 2, F, B), bf16),
            pltpu.VMEM((D, B), f32),
            pltpu.VMEM((D, B), f32),
            pltpu.VMEM((4, 4 * B, B), bf16),
            pltpu.VMEM((4, D, B), f32), pltpu.VMEM((D, 2 * B), f32),
        ],
        compiler_params=pltpu.CompilerParams(vmem_limit_bytes=100 * 1024 * 1024),
    )(qT, kT, vT, A_shift_k.T, A_ssm_k, A_ssm_D, B_w1, B_w2.T, Fm, Gm)
    return outT.T[None]
```

```python
import jax
import jax.numpy as jnp
import numpy as np
import jax.experimental.pallas as pl
import jax.experimental.pallas.tpu as pltpu

D, S, F = 448, 2048, 1792
B = 128
NB = S // B
NS = NB // 2
NF = F // B
NU = 28
L2 = 4
CH = D // NU
DR = D // 4
f32, bf16, u32 = jnp.float32, jnp.bfloat16, jnp.uint32


def _dft_mats():
    n = np.arange(B)[:, None].astype(np.float64)
    w = 2 * np.pi * (np.arange(B)[None, :] + 0.5) / (2 * B)
    sig = np.where(np.arange(B) % 2 == 0, 1.0, -1.0)[None, :]
    re, im = np.cos(w * n), -np.sin(w * n) * sig
    return (np.stack([re, im]).astype(np.float32),
            (np.concatenate([re.T, im.T], axis=0) / B).astype(np.float32))


_FM, _GM = _dft_mats()


def _ld32(ref, idx, r):
    return ref.bitcast(u32)[(*idx, slice(r.start // 2, r.stop // 2), slice(None))]


def _ldb(ref, idxs, r, axis):
    parts = [_ld32(ref, i, r) for i in idxs]
    return pltpu.bitcast(parts[0] if len(parts) == 1 else jnp.concatenate(parts, axis=axis), bf16)


def _kernel(qT_h, kT_h, vT_h, skT_h, ssmk_h, sD_h, w1_h, w2T_h, Fm_h, Gm_h, oT_h,
            qb, kb, vb, sb, w1b, w2b, ob, skT, sD, Fm, Gm, sems,
            w1T, skb, db, Ua, Ub, Us, Ka, Kb, Kc, hT, Kpr, Kpi, xnb, yb, acc, f0):
    def cp_blk(src, dst, i, sem):
        return pltpu.make_async_copy(src.at[:, pl.ds(B * i, B)], dst.at[i], sems.at[sem])

    def cp_in(n, i):
        src, dst = ((qT_h, qb), (kT_h, kb), (vT_h, vb), (ssmk_h, sb))[n]
        return cp_blk(src, dst, i, 4 * i + n)

    def cp_out(i):
        return pltpu.make_async_copy(ob.at[i], oT_h.at[:, pl.ds(B * i, B)], sems.at[92 + i])

    W1 = lambda *cs: [cp_blk(w1_h, w1b, c, 64 + c) for c in cs]
    W2 = lambda *cs: [cp_blk(w2T_h, w2b, c, 78 + c) for c in cs]
    KVS = lambda *bs: [cp_in(n, i) for n in (1, 2, 3) for i in bs]
    Q = lambda *bs: [cp_in(0, i) for i in bs]
    small = [pltpu.make_async_copy(src, dst, sems.at[108 + n]) for n, (src, dst) in
             enumerate(((skT_h, skT), (sD_h, sD), (Fm_h, Fm), (Gm_h, Gm)))]

    batches = {
        -1: Q(0, 1) + W1(0, 1, 2, 3, 4, 5) + W2(0, 1) + W1(6, 7) + W2(2, 3) + W1(8, 9),
        0: W2(4, 5) + W1(10, 11) + W2(6, 7),
        4: W1(12, 13) + W2(8, 9),
        8: Q(2, 3) + W2(10, 11, 12, 13),
        12: small + KVS(0, 1),
        16: KVS(2, 3),
        24: Q(4, 5) + KVS(4, 5),
    }
    for s in range(1, NS - 2):
        batches[NU * s + (L2 if s > 1 else 8)] = Q(2 * s + 4, 2 * s + 5) + KVS(2 * s + 4, 2 * s + 5)
    for c in batches[-1]:
        c.start()

    lane = jax.lax.broadcasted_iota(jnp.int32, (CH // 2, B), 1)
    blk = slice(0, B)

    def smallprep():
        sk = skT[...].astype(f32)
        for j in range(4):
            skb[j] = jnp.broadcast_to(sk[j:j + 1, :], (B, D)).T
        db[...] = jnp.broadcast_to(sD[...].astype(f32)[None, :], (B, D)).T

    def ln(i):
        x = qb[i].astype(f32)
        mu = jnp.sum(x, axis=0, keepdims=True) * (1.0 / D)
        xc = x - mu
        var = jnp.sum(xc * xc, axis=0, keepdims=True) * (1.0 / D)
        xnb[i % 4, :D, :] = (xc * jax.lax.rsqrt(var + 1e-5)).astype(bf16)

    def fmat():
        return jnp.concatenate([_ldb(Fm, [(0,)], blk, 1), _ldb(Fm, [(1,)], blk, 1)], axis=1)

    def dft_kv(s, u):
        r = slice(CH * u, CH * (u + 1))
        kvs = []
        for b in range(2):
            i = 2 * s + b
            a0 = _ld32(kb, (i,), r)
            ap = _ld32(kb, (i - 1,), r) if i > 0 else jnp.zeros_like(a0)
            ks = pltpu.bitcast(a0, bf16).astype(f32) * skb[0, r, :]
            for j in range(1, 4):
                m = pltpu.roll(jnp.where(lane >= B - j, ap, a0), j, 1)
                ks = ks + pltpu.bitcast(m, bf16).astype(f32) * skb[j, r, :]
            kvs.append(ks * vb[i, r, :].astype(f32))
        T = jnp.dot(jnp.concatenate(kvs, axis=0).astype(bf16), fmat(), preferred_element_type=f32)
        for b in range(2):
            i = 2 * s + b
            ur, ui = T[b * CH:(b + 1) * CH, :B], T[b * CH:(b + 1) * CH, B:]
            Ua[i, r, :] = ur
            Ub[i, r, :] = ui
            Us[i, r, :] = ur + ui

    def dft_k(s, u):
        r = slice(CH * u, CH * (u + 1))
        T = jnp.dot(_ldb(sb, [(2 * s,), (2 * s + 1,)], r, 0), fmat(), preferred_element_type=f32)
        for b in range(2):
            i = 2 * s + b
            kr, ki = T[b * CH:(b + 1) * CH, :B], T[b * CH:(b + 1) * CH, B:]
            if i == 0:
                kr = kr + db[r, :]
                c, d = kr, ki
            elif b == 0:
                c, d = kr - Kpi[r, :], ki + Kpr[r, :]
            else:
                c, d = kr - pki, ki + pkr
            pkr, pki = kr, ki
            Ka[i, r, :] = c
            Kb[i, r, :] = d - c
            Kc[i, r, :] = c + d
        Kpr[r, :] = pkr
        Kpi[r, :] = pki

    def mac(s, g):
        r = slice(8 * g, 8 * (g + 1))
        terms = [[], []]
        k1 = (Ka[2 * s + 1, r, :], Kb[2 * s + 1, r, :], Kc[2 * s + 1, r, :])
        for j in range(2 * s + 2):
            ua, ub, us = Ua[j, r, :], Ub[j, r, :], Us[j, r, :]
            terms[1].append((k1[0] * us, k1[1] * ua, k1[2] * ub))
            m0 = 2 * s - j
            if m0 >= 0:
                k1 = (Ka[m0, r, :], Kb[m0, r, :], Kc[m0, r, :])
                terms[0].append((k1[0] * us, k1[1] * ua, k1[2] * ub))
        a = []
        for ts in terms:
            t0 = ts[0]
            for t1 in ts[1:]:
                t0 = tuple(p + q for p, q in zip(t0, t1))
            a.append(t0)
        yr = jnp.concatenate([a[b][0] - a[b][2] for b in range(2)], axis=0)
        yi = jnp.concatenate([a[b][0] + a[b][1] for b in range(2)], axis=0)
        lhs = jnp.concatenate([yr, yi], axis=1).astype(bf16)
        y = jnp.dot(lhs, _ldb(Gm, [()], slice(0, 2 * B), 0), preferred_element_type=f32)
        for b in range(2):
            yb[(2 * s + b) % 4, r, :] = y[8 * b:8 * (b + 1), :]

    def ffn1(s, u):
        b = u % 2
        r = slice(B * (u // 2), B * (u // 2 + 1))
        lhs = _ldb(w1T, [(k,) for k in range(4)], r, 1)
        rhs = _ldb(xnb, [((2 * s + b) % 4,)], slice(0, 4 * B), 0)
        hh = jnp.dot(lhs, rhs, preferred_element_type=f32)
        hT[s % 2, b, r, :] = (hh + hh * jnp.tanh(hh)).astype(bf16)

    def finish(i, r, tot):
        x = qb[i, r, :].astype(f32)
        xn = xnb[i % 4, r, :].astype(f32)
        ob[i, r, :] = (x + xn * yb[i % 4, r, :] + tot).astype(bf16)

    def ffn2(s, u):
        kc, q = u // 4, u % 4
        r = slice(DR * q, DR * (q + 1))
        lhs = _ldb(w2b, [(2 * kc,), (2 * kc + 1,)], r, 1)
        rhs = _ldb(hT, [(s % 2, 0), (s % 2, 1)], slice(2 * B * kc, 2 * B * (kc + 1)), 1)
        p = jnp.dot(lhs, rhs, preferred_element_type=f32)
        if kc == 0:
            acc[r, :] = p
        elif kc < 6:
            acc[r, :] = acc[r, :] + p
        elif s == 0:
            f0[r, :] = acc[r, :] + p
        else:
            for b in range(2):
                finish(2 * s + b, r, acc[r, b * B:(b + 1) * B] + p[:, b * B:(b + 1) * B])

    def final0(q):
        r = slice(DR * q, DR * (q + 1))
        for i in range(2):
            finish(i, r, f0[r, i * B:(i + 1) * B])
        if q == 3:
            cp_out(0).start()
            cp_out(1).start()

    def w1prep(c):
        for k in range(4):
            w = w1b[c, B * k:min(B * (k + 1), D), :].astype(f32) * 0.5
            if k == 3:
                w = jnp.concatenate([w, jnp.zeros((4 * B - D, B), f32)], axis=0)
            w1T[k, B * c:B * (c + 1), :] = w.T.astype(bf16)

    T = NU * NS + L2
    ev = [dict(bar=[], pre=[], m0=[], a=[], b=[], f2=[], m1=[]) for _ in range(T)]

    def at(t, slot, fn, *args):
        ev[t][slot].append((fn, args))

    for k in range(7):
        ev[4 * k]['bar'] = W1(2 * k, 2 * k + 1) + (W2(2 * k - 4, 2 * k - 3) if k >= 2 else [])
        at(4 * k, 'pre', w1prep, 2 * k)
        at(4 * k, 'pre', w1prep, 2 * k + 1)
    ev[24]['bar'] += Q(2, 3)
    ev[NU]['bar'] = W2(10, 11, 12, 13)
    ev[NU + 8]['bar'] = small + KVS(0, 1)
    at(NU + 8, 'pre', smallprep)
    ev[NU + 14]['bar'] = KVS(2, 3)
    ev[NU + 20]['bar'] = Q(4, 5) + KVS(4, 5)
    for s in range(2, NS):
        bar = (Q(2 * s + 2, 2 * s + 3) + KVS(2 * s + 2, 2 * s + 3)) if s + 1 < NS else []
        ev[NU * s + L2]['bar'] = bar + [cp_out(2 * s - 4), cp_out(2 * s - 3)]
    for c in range(NU):
        td = [NU + 8 + c // 4, NU + 14 + c // 4, NU + 20 + c // 3]
        td += [NU * (s - 1) + L2 + c for s in range(3, NS)]
        for s in range(NS):
            at(td[s], 'a', dft_kv, s, c)
            at(td[s], 'b', dft_k, s, c)
    for c in range(NU):
        tm = [NU + 9 + c // 4, NU + 15 + c // 2] + [NU * s + c for s in range(2, NS)]
        for s in range(NS):
            at(tm[s], 'm0', mac, s, 2 * c)
            at(tm[s], 'm1', mac, s, 2 * c + 1)
    for q in range(4):
        at(NU + 18 + q, 'b', final0, q)
    for s in range(NS):
        for u in range(NU):
            ev[NU * s + u + (L2 if s > 0 else 8)]['f2'].append((s, u))

    for i in range(4):
        xnb[i, D:, :] = jnp.zeros((4 * B - D, B), bf16)
    for c in Q(0, 1):
        c.wait()
    ln(0)
    ln(1)
    for t in range(T):
        s, u = t // NU, t % NU
        e = ev[t]

        def run(slot):
            for fn, args in e[slot]:
                fn(*args)

        def run_ffn2():
            for s2, u2 in e['f2']:
                ffn2(s2, u2)
                if u2 == NU - 1 and s2 > 0:
                    cp_out(2 * s2).start()
                    cp_out(2 * s2 + 1).start()

        for c in e['bar']:
            c.wait()
        for c in batches.get(t, []):
            c.start()
        run('pre')
        early2 = s == 0 and u % 4 == 0
        if early2:
            run_ffn2()
        if s < NS:
            ffn1(s, u)
        run('m0')
        run('a')
        run('b')
        if not early2:
            run_ffn2()
        run('m1')
        if u == NU - 1 and s + 1 < NS:
            ln(2 * s + 2)
            ln(2 * s + 3)
    for i in range(NB - 4, NB):
        cp_out(i).wait()


@jax.jit
def pallas_parallel_sum__ssm_conv_h3__dense_activation_silu__prompt_kernel(
    A_q: jax.Array,
    A_k: jax.Array,
    A_v: jax.Array,
    A_shift_k: jax.Array,
    A_ssm_k: jax.Array,
    A_ssm_D: jax.Array,
    B_x: jax.Array,
    B_w1: jax.Array,
    B_w2: jax.Array,
):
    hbm = pl.BlockSpec(memory_space=pltpu.HBM)
    blocks = lambda n: pltpu.VMEM((n, D, B), bf16)
    outT = pl.pallas_call(
        _kernel,
        in_specs=[hbm] * 10,
        out_specs=hbm,
        out_shape=jax.ShapeDtypeStruct((D, S), A_q.dtype),
        scratch_shapes=[
            blocks(NB), blocks(NB), blocks(NB), blocks(NB), blocks(NF), blocks(NF), blocks(NB),
            pltpu.VMEM((4, D), bf16), pltpu.VMEM((D,), bf16),
            pltpu.VMEM((2, B, B), bf16), pltpu.VMEM((2 * B, B), bf16),
            pltpu.SemaphoreType.DMA((112,)),
            pltpu.VMEM((4, F, B), bf16),
            pltpu.VMEM((4, D, B), f32),
            pltpu.VMEM((D, B), f32),
        ] + [pltpu.VMEM((NB, D, B), f32)] * 6 + [
            pltpu.VMEM((2, 2, F, B), bf16),
            pltpu.VMEM((D, B), f32),
            pltpu.VMEM((D, B), f32),
            pltpu.VMEM((4, 4 * B, B), bf16),
            pltpu.VMEM((4, D, B), f32),
            pltpu.VMEM((D, 2 * B), f32),
            pltpu.VMEM((D, 2 * B), f32),
        ],
        compiler_params=pltpu.CompilerParams(
            vmem_limit_bytes=100 * 1024 * 1024,
            flags={"XLA_TPU_EVENLY_DISTRIBUTE_CRITICAL_NODES": True}),
    )(A_q[0].T, A_k[0].T, A_v[0].T, A_shift_k.T, A_ssm_k, A_ssm_D, B_w1, B_w2.T,
      jnp.asarray(_FM, dtype=bf16), jnp.asarray(_GM, dtype=bf16))
    return outT.T[None]
```
